```python
import os as _os
_os.environ.setdefault("JAX_PLATFORMS", "cpu")
import jax
import jax.numpy as jnp

def _softmax(x, axis=-1):
    return jax.nn.softmax(x, axis=axis)
def _gelu(x):
    return jax.nn.gelu(x, approximate=True)
def _silu(x):
    return jax.nn.silu(x)
def _sigmoid(x):
    return jax.nn.sigmoid(x)
def _layernorm(x, axis=-1, eps=1e-5):
    m = jnp.mean(x, axis=axis, keepdims=True)
    v = jnp.var(x, axis=axis, keepdims=True)
    return (x - m) / jnp.sqrt(v + eps)
def _scatter_add(tgt, idx, src, axis=0):
    return tgt.at[idx].add(src)
def _segment_sum(src, seg, n):
    return jax.ops.segment_sum(src, seg, n)
class _Rng:
    def __init__(self, key):
        self._k = key
    def _next(self):
        self._k, sub = jax.random.split(self._k)
        return sub
    def normal(self, shape):
        return jax.random.normal(self._next(), shape, dtype=jnp.bfloat16)
    def randint(self, lo, hi, shape):
        return jax.random.randint(self._next(), shape, lo, hi, dtype=jnp.int32)
    def uniform(self, shape, lo=0.0, hi=1.0):
        return jax.random.uniform(self._next(), shape, jnp.bfloat16, lo, hi)
    def permutation(self, n):
        return jax.random.permutation(self._next(), n)


kernel_name = 'standalone__mha_softmax__near_ridge'

def setup_inputs():
    _rng = _Rng(jax.random.key(int.from_bytes(__import__("os").urandom(4), "little")))
    _w = (lambda a: (lambda t: t.astype(jnp.bfloat16) if jnp.issubdtype(t.dtype, jnp.floating) else t)(jnp.asarray(a)))
    B, H, Sq, Sk, D = 16, 16, 256, 256, 256
    return {
        "q": _w((lambda *s: _rng.normal(s) * 0.4)(B, H, Sq, D)),
        "k": _w((lambda *s: _rng.normal(s) * 0.4)(B, H, Sk, D)),
        "v": _w((lambda *s: _rng.normal(s) * 0.05)(B, H, Sk, D)),
    }

def reference(q, k, v):
    scale = q.shape[-1] ** -0.5
    scores = jnp.einsum("bhqd,bhkd->bhqk", q, k) * scale
    p = _softmax(scores, axis=-1)
    return jnp.einsum("bhqk,bhkd->bhqd", p, v)
```

```python
import jax
import jax.numpy as jnp
from jax import lax
import jax.experimental.pallas as pl
import jax.experimental.pallas.tpu as pltpu

CH = 4
WINDOW = 3
TAIL = 1


def _attend(q, k, v, scale):
    s = lax.dot_general(q, k, (((1,), (1,)), ((), ())),
                        preferred_element_type=jnp.float32)
    s = s * scale
    m = jnp.max(s, axis=1, keepdims=True)
    p = jnp.exp(s - m)
    l = jnp.sum(p, axis=1, keepdims=True)
    o = jnp.dot(p.astype(v.dtype), v, preferred_element_type=jnp.float32)
    return o * (1.0 / l)


@jax.jit
def pallas_standalone__mha_softmax__near_ridge_kernel(
    q: jax.Array,
    k: jax.Array,
    v: jax.Array,
):
    B, H, Sq, D = q.shape
    Sk = k.shape[2]
    N = B * H
    scale = D ** -0.5
    ch = CH
    nch = N // ch
    nb = nch - TAIL
    ring = WINDOW + 1

    def kernel_function(q_hbm, k_hbm, v_hbm, o_hbm, qb, kb, vb, rsem, wsem):
        def reads(i):
            sl = pl.ds(i * ch, ch)
            sem = rsem.at[i % ring]
            return [pltpu.make_async_copy(src.at[sl], dst.at[sl], sem)
                    for src, dst in ((q_hbm, qb), (k_hbm, kb), (v_hbm, vb))]

        def write(h0, nh, j):
            sl = pl.ds(h0, nh)
            return pltpu.make_async_copy(qb.at[sl], o_hbm.at[sl], wsem.at[j])

        def compute(i):
            for h in range(ch):
                hh = i * ch + h
                o = _attend(qb[hh], kb[hh], vb[hh], scale)
                qb[hh] = o.astype(qb.dtype)

        for j in range(WINDOW):
            for c in reads(j):
                c.start()

        def read_body(i, _):
            @pl.when(i + WINDOW < nch)
            def _():
                for c in reads(i + WINDOW):
                    c.start()
            for c in reads(i):
                c.wait()
            compute(i)

        lax.fori_loop(0, nb, read_body, None)

        big = write(0, nb * ch, 0)
        big.start()
        for j in range(nb, nch):
            for c in reads(j):
                c.wait()

        def tail_body(i, _):
            compute(i)
            write(i * ch, ch, 1).start()

        lax.fori_loop(nb, nch, tail_body, None)

        big.wait()
        for j in range(nb, nch):
            write(j * ch, ch, 1).wait()

    hbm = pl.BlockSpec(memory_space=pl.ANY)
    out = pl.pallas_call(
        kernel_function,
        in_specs=[hbm, hbm, hbm],
        out_specs=hbm,
        out_shape=jax.ShapeDtypeStruct((N, Sq, D), q.dtype),
        scratch_shapes=[
            pltpu.VMEM((N, Sq, D), q.dtype),
            pltpu.VMEM((N, Sk, D), k.dtype),
            pltpu.VMEM((N, Sk, D), v.dtype),
            pltpu.SemaphoreType.DMA((ring,)),
            pltpu.SemaphoreType.DMA((2,)),
        ],
        compiler_params=pltpu.CompilerParams(vmem_limit_bytes=127 * 2**20),
    )(q.reshape(N, Sq, D), k.reshape(N, Sk, D), v.reshape(N, Sk, D))
    return out.reshape(B, H, Sq, D)
```

```python
import jax
import jax.numpy as jnp
from jax import lax
import jax.experimental.pallas as pl
import jax.experimental.pallas.tpu as pltpu

HG = 4
WINDOW = 3
WROWS = 16
TAIL = 1
TSPLIT = 4


def _attend(q, k, v, scale):
    s = lax.dot_general(q, k, (((1,), (1,)), ((), ())),
                        preferred_element_type=jnp.float32)
    s = s * scale
    m = jnp.max(s, axis=1, keepdims=True)
    p = jnp.exp(s - m)
    l = jnp.sum(p, axis=1, keepdims=True)
    o = jnp.dot(p.astype(v.dtype), v, preferred_element_type=jnp.float32)
    return o * (1.0 / l)


@jax.jit
def pallas_standalone__mha_softmax__near_ridge_kernel(
    q: jax.Array,
    k: jax.Array,
    v: jax.Array,
):
    B, H, Sq, D = q.shape
    Sk = k.shape[2]
    scale = D ** -0.5
    ng = (B * H) // HG
    gq = HG * Sq
    gk = HG * Sk
    nb = ng - TAIL
    ring = WINDOW + 1

    def kernel_function(q_hbm, k_hbm, v_hbm, o_hbm, qb, kb, vb, rsem, wsem):
        def reads(i):
            sl = pl.ds(i, 1)
            sem = rsem.at[i % ring]
            return [pltpu.make_async_copy(src.at[sl], dst.at[sl], sem)
                    for src, dst in ((q_hbm, qb), (k_hbm, kb), (v_hbm, vb))]

        def main_writes():
            out = []
            for j in range(gq // WROWS):
                idx = (pl.ds(0, nb), pl.ds(j * WROWS, WROWS))
                out.append(pltpu.make_async_copy(qb.at[idx], o_hbm.at[idx],
                                                 wsem.at[0]))
            return out

        def tail_writes(i):
            r = gq // TSPLIT
            out = []
            for j in range(TSPLIT):
                idx = (pl.ds(i, 1), pl.ds(j * r, r))
                out.append(pltpu.make_async_copy(qb.at[idx], o_hbm.at[idx],
                                                 wsem.at[1]))
            return out

        def compute(i):
            for h in range(HG):
                sq = pl.ds(h * Sq, Sq)
                sk = pl.ds(h * Sk, Sk)
                o = _attend(qb[i, sq, :], kb[i, sk, :], vb[i, sk, :], scale)
                qb[i, sq, :] = o.astype(qb.dtype)

        for j in range(WINDOW):
            for c in reads(j):
                c.start()

        def read_body(i, _):
            @pl.when(i + WINDOW < ng)
            def _():
                for c in reads(i + WINDOW):
                    c.start()
            for c in reads(i):
                c.wait()
            compute(i)

        lax.fori_loop(0, nb, read_body, None)

        for c in main_writes():
            c.start()
        for j in range(nb, ng):
            for c in reads(j):
                c.wait()

        def tail_body(i, _):
            compute(i)
            for c in tail_writes(i):
                c.start()

        lax.fori_loop(nb, ng, tail_body, None)

        for c in main_writes():
            c.wait()
        for j in range(nb, ng):
            for c in tail_writes(j):
                c.wait()

    hbm = pl.BlockSpec(memory_space=pl.ANY)
    out = pl.pallas_call(
        kernel_function,
        in_specs=[hbm, hbm, hbm],
        out_specs=hbm,
        out_shape=jax.ShapeDtypeStruct((ng, gq, D), q.dtype),
        scratch_shapes=[
            pltpu.VMEM((ng, gq, D), q.dtype),
            pltpu.VMEM((ng, gk, D), k.dtype),
            pltpu.VMEM((ng, gk, D), v.dtype),
            pltpu.SemaphoreType.DMA((ring,)),
            pltpu.SemaphoreType.DMA((2,)),
        ],
        compiler_params=pltpu.CompilerParams(vmem_limit_bytes=127 * 2**20),
    )(q.reshape(ng, gq, D), k.reshape(ng, gk, D), v.reshape(ng, gk, D))
    return out.reshape(B, H, Sq, D)
```

```python
import jax
import jax.numpy as jnp
from jax import lax
import jax.experimental.pallas as pl
import jax.experimental.pallas.tpu as pltpu

CH = 4
GH = 32
WROWS = 16
TAIL = 5


def _attend(q, k, v, scale):
    s = lax.dot_general(q, k, (((1,), (1,)), ((), ())),
                        preferred_element_type=jnp.float32)
    s = s * scale
    m = jnp.max(s, axis=1, keepdims=True)
    p = jnp.exp(s - m)
    l = jnp.sum(p, axis=1, keepdims=True)
    o = jnp.dot(p.astype(v.dtype), v, preferred_element_type=jnp.float32)
    return o * (1.0 / l)


@jax.jit
def pallas_standalone__mha_softmax__near_ridge_kernel(
    q: jax.Array,
    k: jax.Array,
    v: jax.Array,
):
    B, H, Sq, D = q.shape
    Sk = k.shape[2]
    Dv = v.shape[3]
    N = B * H
    scale = D ** -0.5
    assert Dv == D and q.dtype == k.dtype == v.dtype
    assert N % GH == 0 and GH % CH == 0 and CH < TAIL < 2 * CH
    assert (Sq % WROWS == 0) and (Sk % 16 == 0)

    ng = N // GH
    cpg = GH // CH
    nch = N // CH
    nloop = nch - 2
    gq, gk = GH * Sq, GH * Sk
    cq, ck = CH * Sq, CH * Sk
    tail_rows = TAIL * Sq
    wsem = nch % 2

    def kernel_function(q_hbm, k_hbm, v_hbm, o_hbm, qb, kb, vb, sem):
        def locate(i):
            return i // cpg, i % cpg

        def rows(c, n):
            start = c * n
            return start if isinstance(start, int) else pl.multiple_of(start, n)

        def reads(i):
            g, c = locate(i)
            out = []
            for src, dst, n in ((q_hbm, qb, cq), (k_hbm, kb, ck), (v_hbm, vb, ck)):
                idx = (pl.ds(g, 1), pl.ds(rows(c, n), n))
                out.append(pltpu.make_async_copy(src.at[idx], dst.at[idx],
                                                 sem.at[i % 2]))
            return out

        def main_writes():
            out = []
            for j in range(gq // WROWS):
                n = ng if (j + 1) * WROWS <= gq - tail_rows else ng - 1
                if n == 0:
                    continue
                idx = (pl.ds(0, n), pl.ds(j * WROWS, WROWS))
                out.append(pltpu.make_async_copy(qb.at[idx], o_hbm.at[idx],
                                                 sem.at[wsem]))
            return out

        def tail_write():
            idx = (pl.ds(ng - 1, 1), pl.ds(gq - tail_rows, tail_rows))
            return pltpu.make_async_copy(qb.at[idx], o_hbm.at[idx], sem.at[wsem])

        def head(i, h):
            g, c = locate(i)
            first = c * CH + h
            sq = pl.ds(rows(first, Sq), Sq)
            sk = pl.ds(rows(first, Sk), Sk)
            o = _attend(qb[g, sq, :], kb[g, sk, :], vb[g, sk, :], scale)
            qb[g, sq, :] = o.astype(qb.dtype)

        for i in range(2):
            for c in reads(i):
                c.start()

        def read_body(i, _):
            for c in reads(i):
                c.wait()
            for c in reads(i + 2):
                c.start()
            for h in range(CH):
                head(i, h)

        lax.fori_loop(0, nloop, read_body, None)

        started = False
        for i in range(nloop, nch):
            for c in reads(i):
                c.wait()
            for h in range(CH):
                if not started and i * CH + h >= N - TAIL:
                    for c in main_writes():
                        c.start()
                    started = True
                head(i, h)

        tail_write().start()
        for c in main_writes():
            c.wait()
        tail_write().wait()

    hbm = pl.BlockSpec(memory_space=pl.ANY)
    out = pl.pallas_call(
        kernel_function,
        in_specs=[hbm, hbm, hbm],
        out_specs=hbm,
        out_shape=jax.ShapeDtypeStruct((ng, gq, D), q.dtype),
        scratch_shapes=[
            pltpu.VMEM((ng, gq, D), q.dtype),
            pltpu.VMEM((ng, gk, D), k.dtype),
            pltpu.VMEM((ng, gk, D), v.dtype),
            pltpu.SemaphoreType.DMA((2,)),
        ],
        compiler_params=pltpu.CompilerParams(vmem_limit_bytes=104 * 2**20),
    )(q.reshape(ng, gq, D), k.reshape(ng, gk, D), v.reshape(ng, gk, D))
    return out.reshape(B, H, Sq, D)
```
